```python
import jax
import jax.numpy as jnp

def _softmax(x, axis=-1):
    return jax.nn.softmax(x, axis=axis)

def _gelu(x):
    return jax.nn.gelu(x, approximate=True)

def _silu(x):
    return jax.nn.silu(x)

def _sigmoid(x):
    return jax.nn.sigmoid(x)

def _layernorm(x, axis=-1, eps=1e-05):
    m = jnp.mean(x, axis=axis, keepdims=True)
    v = jnp.var(x, axis=axis, keepdims=True)
    return (x - m) / jnp.sqrt(v + eps)

def _scatter_add(tgt, idx, src, axis=0):
    return tgt.at[idx].add(src)

def _segment_sum(src, seg, n):
    return jax.ops.segment_sum(src, seg, n)

class _Rng:

    def __init__(self, key):
        self._k = key

    def _next(self):
        self._k, sub = jax.random.split(self._k)
        return sub

    def normal(self, shape):
        return jax.random.normal(self._next(), shape, dtype=jnp.bfloat16)

    def randint(self, lo, hi, shape):
        return jax.random.randint(self._next(), shape, lo, hi, dtype=jnp.int32)

    def uniform(self, shape, lo=0.0, hi=1.0):
        return jax.random.uniform(self._next(), shape, jnp.bfloat16, lo, hi)

    def permutation(self, n):
        return jax.random.permutation(self._next(), n)
kernel_name = 'adaLN_cond__sliding_block_cached__glu_gated_bilinear__decode'

def setup_inputs():
    _rng = _Rng(jax.random.key(int.from_bytes(__import__("os").urandom(4), "little")))
    _w = lambda a: (lambda t: t.astype(jnp.bfloat16) if jnp.issubdtype(t.dtype, jnp.floating) else t)(jnp.asarray(a))

    def _A_setup():
        B, Sq, D = (1, 1, 640)
        Hq, Hkv, Sk, Dh = (32, 32, 32768, 192)
        assert Hq % Hkv == 0, (Hq, Hkv)
        return {'x': _w((lambda *s: _rng.normal(s) * 0.05)(B, Sq, D)), 'k_cache': _w((lambda *s: _rng.normal(s) * 0.05)(B, Hkv, Sk, Dh)), 'v_cache': _w((lambda *s: _rng.normal(s) * 0.05)(B, Hkv, Sk, Dh)), 'wq': _w((lambda *s: _rng.normal(s) * 0.05)(D, Hq * Dh) * D ** (-0.5)), 'wo': _w((lambda *s: _rng.normal(s) * 0.05)(Hq * Dh, D) * (Hq * Dh) ** (-0.5))}
    _A_in = _A_setup()

    def _B_setup():
        B, S, D, F = (1, 1, 640, 1536)
        return {'x': _w((lambda *s: _rng.normal(s) * 0.05)(B, S, D)), 'w_gate': _w((lambda *s: _rng.normal(s) * 0.05)(D, F) * D ** (-0.5)), 'w_up': _w((lambda *s: _rng.normal(s) * 0.05)(D, F) * D ** (-0.5)), 'w_down': _w((lambda *s: _rng.normal(s) * 0.05)(F, D) * F ** (-0.5))}
    _B_in = _B_setup()
    return {'A_x': _A_in['x'], 'A_k_cache': _A_in['k_cache'], 'A_v_cache': _A_in['v_cache'], 'A_wq': _A_in['wq'], 'A_wo': _A_in['wo'], 'B_x': _B_in['x'], 'B_w_gate': _B_in['w_gate'], 'B_w_up': _B_in['w_up'], 'B_w_down': _B_in['w_down'], 'c': _w((lambda *s: _rng.normal(s) * 0.05)(1, 640)), 'w_mod': _w((lambda *s: _rng.normal(s) * 0.05)(640, 6 * 640) * 640 ** (-0.5))}

def reference(A_x, A_k_cache, A_v_cache, A_wq, A_wo, B_x, B_w_gate, B_w_up, B_w_down, c, w_mod):

    def _A_ref(x, k_cache, v_cache, wq, wo):
        B, Sq, D = x.shape
        Hq, Dh = (32, 192)
        Hkv, Sk = (k_cache.shape[1], k_cache.shape[2])
        W = min(4096, max(256, Sk // 4))
        rep = Hq // Hkv
        q = (lambda x, *d: x.transpose(*d))((x @ wq).reshape(B, Sq, Hq, Dh), 0, 2, 1, 3)
        k = jnp.repeat(k_cache[:, :, Sk - W:, :], rep, axis=1)
        v = jnp.repeat(v_cache[:, :, Sk - W:, :], rep, axis=1)
        scores = jnp.einsum('bhqd,bhkd->bhqk', q, k) * Dh ** (-0.5)
        p = _softmax(scores, axis=-1)
        o = jnp.einsum('bhqk,bhkd->bhqd', p, v)
        return (lambda x, *d: x.transpose(*d))(o, 0, 2, 1, 3).reshape(B, Sq, Hq * Dh) @ wo

    def _B_ref(x, w_gate, w_up, w_down):
        g = jnp.einsum('bsd,df->bsf', x, w_gate)
        u = jnp.einsum('bsd,df->bsf', x, w_up)
        h = g * u
        return jnp.einsum('bsf,fd->bsd', h, w_down)
    x = A_x
    mod = (_silu(c) @ w_mod).reshape(c.shape[0], 6, 1, -1)
    sa, ca, ga, sb, cb, gb = (mod[:, 0].copy(), mod[:, 1].copy(), mod[:, 2].copy(), mod[:, 3].copy(), mod[:, 4].copy(), mod[:, 5].copy())
    h = _layernorm(x, axis=-1) * (1 + ca) + sa
    x = x + ga * _A_ref(h, A_k_cache, A_v_cache, A_wq, A_wo)
    h = _layernorm(x, axis=-1) * (1 + cb) + sb
    x = x + gb * _B_ref(h, B_w_gate, B_w_up, B_w_down)
    return x
```

```python
import jax
import jax.numpy as jnp
import numpy as np
import jax.experimental.pallas as pl
import jax.experimental.pallas.tpu as pltpu

D = 640
H = 32
DH = 192
SK = 32768
W = 4096
F = 1536
HD = H * DH
PR = 2 * DH
NP = H // 2
R = 8


def pieces(nrows, ncols, r, c, order='ba'):
    na, nb = nrows // r, ncols // c
    assert na * r == nrows and nb * c == ncols
    if order == 'ba':
        return [(a * r, b * c) for b in range(nb) for a in range(na)]
    return [(a * r, b * c) for a in range(na) for b in range(nb)]


def chunks(lst, n):
    return [lst[i:i + n] for i in range(0, len(lst), n)]


def make(LA=3, NC=4, kvp=(8, 1024), wmp=(8, 768, 'ba'), wqp=(8, 1024, 'ba'), wop=(8, 640), wgp=(8, 768, 'ba'), wdp=(8, 640),
         G=48, wd_chunks=3, pk=0, TA=1):
    f32 = jnp.float32
    bf16 = jnp.bfloat16
    CW = W // NC
    NS = 2 * NC + 1
    WDC = F // wd_chunks

    def kernel(x_hbm, c_hbm, k_hbm, v_hbm, wq_hbm, wo_hbm, wg_hbm, wu_hbm, wd_hbm, wm_hbm,
               out_ref,
               x_v, c_v, kbuf, vbuf, wq_v, wo_v, wg_v, wu_v, wd_v, wm_v,
               ksem, vsem, wsem, wdsem):
        cnt = [0]

        def issue(src, dst, sem, plist, r, c, src_row0=0, src_col0=0, dst_row0=0, dst_col0=0):
            for (r0, c0) in plist:
                p = (r0 // r) % 2 if pk == 0 else cnt[0] % 2
                cnt[0] += 1
                pltpu.make_async_copy(
                    src.at[pl.ds(src_row0 + r0, r), pl.ds(src_col0 + c0, c)],
                    dst.at[pl.ds(dst_row0 + r0, r), pl.ds(dst_col0 + c0, c)], sem).start(priority=p)

        def whole_wait(ref, sem):
            pltpu.make_async_copy(ref, ref, sem).wait()

        def issue_step(j, s):
            row0 = pl.multiple_of(j * PR, 128)
            if s < NC:
                issue(k_hbm, kbuf, ksem.at[s], pieces(PR, CW, *kvp), *kvp, src_row0=row0, src_col0=SK - W + s * CW, dst_col0=s * CW)
            elif s < 2 * NC:
                t = s - NC
                issue(v_hbm, vbuf, vsem.at[t], pieces(PR, CW, *kvp), *kvp, src_row0=row0, src_col0=SK - W + t * CW, dst_col0=t * CW)
            else:
                issue(wo_hbm, wo_v, wsem.at[4], pieces(PR, D, *wop), *wop, src_row0=row0, dst_row0=row0)

        tail = []
        tail_end = []
        for (hbm, vm, sem) in ((wg_hbm, wg_v, wsem.at[2]), (wu_hbm, wu_v, wsem.at[3])):
            for grp in chunks(pieces(D, F, *wgp), G):
                tail.append((hbm, vm, sem, grp, wgp[:2], len(tail_end)))
            tail_end.append(len(tail))
        for i in range(wd_chunks):
            pl_ = [(r0 + i * WDC, c0) for (r0, c0) in pieces(WDC, D, *wdp)]
            for grp in chunks(pl_, G):
                tail.append((wd_hbm, wd_v, wdsem.at[i], grp, wdp, len(tail_end)))
            tail_end.append(len(tail))
        tail_pos = [0]

        def issue_tail(n=1):
            for _ in range(n):
                if tail_pos[0] < len(tail):
                    hbm, vm, sem, grp, rc, _ = tail[tail_pos[0]]
                    tail_pos[0] += 1
                    issue(hbm, vm, sem, grp, *rc)

        def issue_tail_through(i, extra=0):
            issue_tail(max(0, tail_end[i] - tail_pos[0]) + extra)

        x_cp = pltpu.make_async_copy(x_hbm, x_v, wsem.at[5])
        c_cp = pltpu.make_async_copy(c_hbm, c_v, wsem.at[6])
        wm_groups = chunks(pieces(D, 6 * D, *wmp), G)
        wq_groups = chunks(pieces(D, HD, *wqp), G)
        issue(wm_hbm, wm_v, wsem.at[0], wm_groups[0], *wmp[:2])
        x_cp.start()
        c_cp.start()
        for grp in wm_groups[1:]:
            issue(wm_hbm, wm_v, wsem.at[0], grp, *wmp[:2])
        issue(wq_hbm, wq_v, wsem.at[1], wq_groups[0], *wqp[:2])

        x_cp.wait()
        c_cp.wait()
        x = jnp.broadcast_to(x_v[0].astype(f32), (R, D))
        c = jnp.broadcast_to(c_v[...].astype(f32), (R, D))
        sc = (c * jax.nn.sigmoid(c)).astype(bf16)

        def ln(t):
            m = jnp.mean(t, axis=-1, keepdims=True)
            d = t - m
            v = jnp.mean(d * d, axis=-1, keepdims=True)
            return d * jax.lax.rsqrt(v + 1e-5)

        lx = ln(x)
        whole_wait(wm_v, wsem.at[0])
        mods = []
        gi = 1
        for i in range(6):
            mods.append(jnp.dot(sc, wm_v[:, i * D:(i + 1) * D], preferred_element_type=f32))
            if i in (1, 3):
                issue(wq_hbm, wq_v, wsem.at[1], wq_groups[gi], *wqp[:2])
                gi += 1
        sa, ca, ga, sb, cb, gb = mods
        h = (lx * (1.0 + ca) + sa).astype(bf16)
        for grp in wq_groups[gi:]:
            issue(wq_hbm, wq_v, wsem.at[1], grp, *wqp[:2])
        for s in range(LA - 1):
            issue_step(0, s)
        whole_wait(wq_v, wsem.at[1])
        scale = DH ** -0.5

        prow = jax.lax.broadcasted_iota(jnp.int32, (R, PR), 0)
        pcol = jax.lax.broadcasted_iota(jnp.int32, (R, PR), 1)
        pmask = prow == (pcol >= DH).astype(jnp.int32)

        def pair(j, acc, last):
            def ahead(s):
                n = s + LA - 1
                if n < NS:
                    issue_step(j, n)
                elif last:
                    issue_tail()
                else:
                    issue_step(j + 1, n - NS)

            off = pl.multiple_of(j * PR, 128)
            q = jnp.dot(h, wq_v[:, pl.ds(off, PR)], preferred_element_type=f32)
            qb = jnp.where(pmask, q, 0.0).astype(bf16)
            ss = []
            for s in range(NC):
                ahead(s)
                whole_wait(kbuf.at[:, pl.ds(s * CW, CW)], ksem.at[s])
                ss.append(jnp.dot(qb, kbuf[:, s * CW:(s + 1) * CW], preferred_element_type=f32) * scale)
            m = _fold(jnp.maximum, ss)
            m = jnp.max(m, axis=-1, keepdims=True)
            o = jnp.zeros((R, PR), f32)
            lsum = jnp.zeros((R, CW), f32)
            for s in range(NC):
                e = jnp.exp(ss[s] - m)
                lsum = lsum + e
                p = e.astype(bf16)
                ahead(NC + s)
                whole_wait(vbuf.at[:, pl.ds(s * CW, CW)], vsem.at[s])
                o = o + jax.lax.dot_general(p, vbuf[:, s * CW:(s + 1) * CW], (((1,), (1,)), ((), ())), preferred_element_type=f32)
            l = jnp.sum(lsum, axis=-1, keepdims=True)
            ob = jnp.where(pmask, o / l, 0.0).astype(bf16)
            ahead(2 * NC)
            whole_wait(wo_v.at[pl.ds(off, PR)], wsem.at[4])
            return acc + jnp.dot(ob, wo_v[pl.ds(off, PR), :], preferred_element_type=f32)

        acc = jax.lax.fori_loop(0, NP - 1, lambda j, a: pair(j, a, False), jnp.zeros((R, D), f32))
        acc = pair(NP - 1, acc, True)

        attn = jnp.sum(acc, axis=0, keepdims=True)
        x1 = x + ga * attn
        h2 = (ln(x1) * (1.0 + cb) + sb).astype(bf16)
        issue_tail_through(0, TA)
        whole_wait(wg_v, wsem.at[2])
        g = jnp.dot(h2, wg_v[...], preferred_element_type=f32)
        issue_tail_through(1, TA)
        whole_wait(wu_v, wsem.at[3])
        u = jnp.dot(h2, wu_v[...], preferred_element_type=f32)
        hh = (g * u).astype(bf16)
        y = jnp.zeros((R, D), f32)
        issue_tail(len(tail))
        for i in range(wd_chunks):
            whole_wait(wd_v.at[pl.ds(i * WDC, WDC)], wdsem.at[i])
            y = y + jnp.dot(hh[:, i * WDC:(i + 1) * WDC], wd_v[i * WDC:(i + 1) * WDC, :], preferred_element_type=f32)
        res = x1 + gb * y
        out_ref[...] = res[0:1].astype(out_ref.dtype).reshape(1, 1, D)

    def f(A_x, A_k_cache, A_v_cache, A_wq, A_wo, B_x, B_w_gate, B_w_up, B_w_down, c, w_mod):
        kt = jnp.transpose(A_k_cache, (0, 1, 3, 2)).reshape(HD, SK)
        vt = jnp.transpose(A_v_cache, (0, 1, 3, 2)).reshape(HD, SK)
        any_ = pl.BlockSpec(memory_space=pl.ANY)
        vm = pl.BlockSpec(memory_space=pltpu.VMEM)
        return pl.pallas_call(
            kernel,
            in_specs=[any_] * 10,
            out_specs=vm,
            out_shape=jax.ShapeDtypeStruct((1, 1, D), bf16),
            scratch_shapes=[
                pltpu.VMEM((1, 1, D), bf16), pltpu.VMEM((1, D), bf16),
                pltpu.VMEM((PR, W), bf16), pltpu.VMEM((PR, W), bf16),
                pltpu.VMEM((D, HD), bf16), pltpu.VMEM((HD, D), bf16),
                pltpu.VMEM((D, F), bf16), pltpu.VMEM((D, F), bf16), pltpu.VMEM((F, D), bf16),
                pltpu.VMEM((D, 6 * D), bf16),
                pltpu.SemaphoreType.DMA((NC,)), pltpu.SemaphoreType.DMA((NC,)),
                pltpu.SemaphoreType.DMA((7,)), pltpu.SemaphoreType.DMA((wd_chunks,)),
            ],
            compiler_params=pltpu.CompilerParams(vmem_limit_bytes=100 * 2**20, disable_bounds_checks=True),
        )(A_x, c, kt, vt, A_wq, A_wo, B_w_gate, B_w_up, B_w_down, w_mod)
    return f


def _fold(fn, xs):
    out = xs[0]
    for t in xs[1:]:
        out = fn(out, t)
    return out


_impl = make(G=64, TA=2)


@jax.jit
def pallas_adaLN_cond__sliding_block_cached__glu_gated_bilinear__decode_kernel(
    A_x, A_k_cache, A_v_cache, A_wq, A_wo, B_x, B_w_gate, B_w_up, B_w_down, c, w_mod
):
    return _impl(A_x, A_k_cache, A_v_cache, A_wq, A_wo, B_x, B_w_gate, B_w_up, B_w_down, c, w_mod)
```

```python
import jax
import jax.numpy as jnp
import jax.experimental.pallas as pl
import jax.experimental.pallas.tpu as pltpu

D = 640
H = 32
DH = 192
SK = 32768
WIN = min(4096, max(256, SK // 4))
FF = 1536
HD = H * DH
PR = 2 * DH
NP = H // 2
NB = PR // 128
ROWS = 8

KV_COLS = 1024
AHEAD = 3
TAIL_AHEAD = 100
TAIL_STEP = 64
WD_CHUNKS = 6
WDC = FF // WD_CHUNKS


def _streams(nrows, ncols, r, c, k, row0=0, col0=0):
    na, nb = nrows // r, ncols // c
    per = na // k
    runs = [[(row0 + a * r, col0 + b * c) for a in range(s * per, (s + 1) * per) for b in range(nb)]
            for s in range(k)]
    return [runs[s][i] + (r, c, s % 2) for i in range(per * nb) for s in range(k)]


def _pair_groups():
    groups = []
    for s, kind in enumerate("kv"):
        for blk in range(NB):
            groups.append([(kind, blk, blk * 128 + a * 8, b * KV_COLS, 8, KV_COLS, (a + s) % 2)
                           for b in range(WIN // KV_COLS) for a in range(16)])
    wo = [("w", 0) + p for p in _streams(PR, D, 8, D, 2)]
    riders = range(AHEAD - 1, len(groups))
    per = len(wo) // len(riders)
    for n, gi in enumerate(riders):
        extra = wo[n * per:(n + 1) * per]
        step = 2 * (len(groups[gi]) // (2 * (len(extra) + 1)))
        mixed = []
        for m, piece in enumerate(groups[gi]):
            mixed.append(piece)
            if extra and (m + 1) % step == 0:
                mixed.append(extra.pop(0))
        groups[gi] = mixed + extra
    return groups


_GROUPS = _pair_groups()
_NG = len(_GROUPS)
_LAST_GROUP = {(p[0], p[1]): gi for gi, grp in enumerate(_GROUPS) for p in grp}

_S_MOD_A, _S_MOD_B, _S_WQ, _S_WO, _S_WG, _S_WU, _S_X, _S_C = range(8)


def _layernorm(t):
    mean = jnp.mean(t, axis=-1, keepdims=True)
    d = t - mean
    var = jnp.mean(d * d, axis=-1, keepdims=True)
    return d * jax.lax.rsqrt(var + 1e-5)


def _kernel(x_hbm, c_hbm, k_hbm, v_hbm, wq_hbm, wo_hbm, wg_hbm, wu_hbm, wd_hbm, wm_hbm,
            out_ref,
            x_v, c_v, kbuf, vbuf, wq_v, wo_v, wg_v, wu_v, wd_v, wm_v,
            ksem, vsem, wsem, wdsem):
    f32, bf16 = jnp.float32, jnp.bfloat16

    def start(src, dst, sem, sr, sc, dr, dc, r, c, queue):
        pltpu.make_async_copy(src.at[pl.ds(sr, r), pl.ds(sc, c)],
                              dst.at[pl.ds(dr, r), pl.ds(dc, c)], sem).start(priority=queue)

    def wait_all(ref, sem):
        pltpu.make_async_copy(ref, ref, sem).wait()

    def start_weights(pieces):
        for (hbm, vmem, sem, r0, c0, r, c, queue) in pieces:
            start(hbm, vmem, sem, r0, c0, r0, c0, r, c, queue)

    def weight_pieces(hbm, vmem, sem, *geometry, **origin):
        return [(hbm, vmem, sem) + p for p in _streams(*geometry, **origin)]

    def start_pair_group(j, gi):
        row0 = pl.multiple_of(j * PR, 128)
        for (kind, blk, r0, c0, r, c, queue) in _GROUPS[gi]:
            if kind == "k":
                start(k_hbm, kbuf, ksem.at[blk], row0 + r0, SK - WIN + c0, r0, c0, r, c, queue)
            elif kind == "v":
                start(v_hbm, vbuf, vsem.at[blk], row0 + r0, SK - WIN + c0, r0, c0, r, c, queue)
            else:
                start(wo_hbm, wo_v, wsem.at[_S_WO], row0 + r0, c0, row0 + r0, c0, r, c, queue)

    tail = weight_pieces(wg_hbm, wg_v, wsem.at[_S_WG], D, FF, 8, FF, 8)
    tail_end = {"wg": len(tail)}
    tail += weight_pieces(wu_hbm, wu_v, wsem.at[_S_WU], D, FF, 8, FF, 8)
    tail_end["wu"] = len(tail)
    for i in range(WD_CHUNKS):
        tail += weight_pieces(wd_hbm, wd_v, wdsem.at[i], WDC, D, 8, D, 4, row0=i * WDC)
        tail_end[i] = len(tail)
    tail_pos = [0]

    def start_tail_upto(n):
        n = min(n, len(tail))
        if n > tail_pos[0]:
            start_weights(tail[tail_pos[0]:n])
            tail_pos[0] = n

    def wait_tail(key, ref, sem):
        start_tail_upto(tail_end[key] + TAIL_AHEAD)
        wait_all(ref, sem)

    mod_a = weight_pieces(wm_hbm, wm_v, wsem.at[_S_MOD_A], D, 2 * D, 8, 2 * D, 10)
    mod_b = weight_pieces(wm_hbm, wm_v, wsem.at[_S_MOD_B], D, 4 * D, 8, 2 * D, 10, col0=2 * D)
    wq_pieces = weight_pieces(wq_hbm, wq_v, wsem.at[_S_WQ], D, HD, 8, 1024, 10)
    x_copy = pltpu.make_async_copy(x_hbm, x_v, wsem.at[_S_X])
    c_copy = pltpu.make_async_copy(c_hbm, c_v, wsem.at[_S_C])

    start_weights(mod_a[:8])
    x_copy.start()
    c_copy.start()
    start_weights(mod_a[8:])
    start_weights(wq_pieces[:48])
    x_copy.wait()
    c_copy.wait()
    x = jnp.broadcast_to(x_v[0].astype(f32), (ROWS, D))
    cond = jnp.broadcast_to(c_v[...].astype(f32), (ROWS, D))
    silu_c = (cond * jax.nn.sigmoid(cond)).astype(bf16)
    ln_x = _layernorm(x)
    start_weights(wq_pieces[48:144])
    wait_all(wm_v.at[:, pl.ds(0, 2 * D)], wsem.at[_S_MOD_A])
    shift_a = jnp.dot(silu_c, wm_v[:, 0:D], preferred_element_type=f32)
    scale_a = jnp.dot(silu_c, wm_v[:, D:2 * D], preferred_element_type=f32)
    h = (ln_x * (1.0 + scale_a) + shift_a).astype(bf16)
    start_weights(wq_pieces[144:])
    for gi in range(AHEAD - 1):
        start_pair_group(0, gi)
    start_weights(mod_b)
    wait_all(wq_v, wsem.at[_S_WQ])

    prow = jax.lax.broadcasted_iota(jnp.int32, (ROWS, PR), 0)
    pcol = jax.lax.broadcasted_iota(jnp.int32, (ROWS, PR), 1)
    own_head = prow == (pcol >= DH).astype(jnp.int32)

    def head_pair(j, acc, last):
        started = [AHEAD - 1]
        consumed = set()

        def advance(target):
            while started[0] < target:
                n = started[0]
                if n < _NG:
                    start_pair_group(j, n)
                elif last:
                    start_tail_upto(tail_pos[0] + TAIL_STEP)
                else:
                    assert all(p[:2] in consumed for p in _GROUPS[n - _NG])
                    start_pair_group(j + 1, n - _NG)
                started[0] += 1

        def need(key, ref, sem):
            advance(_LAST_GROUP[key] + AHEAD)
            wait_all(ref, sem)

        def modulation(i):
            return jnp.dot(silu_c, wm_v[:, i * D:(i + 1) * D], preferred_element_type=f32)

        off = pl.multiple_of(j * PR, 128)
        q = jnp.dot(h, wq_v[:, pl.ds(off, PR)], preferred_element_type=f32)
        q = jnp.where(own_head, q, 0.0).astype(bf16)
        mods = []
        s = None
        for b in range(NB):
            rows = pl.ds(b * 128, 128)
            need(("k", b), kbuf.at[rows], ksem.at[b])
            part = jnp.dot(q[:, b * 128:(b + 1) * 128], kbuf[rows, :], preferred_element_type=f32)
            s = part if s is None else s + part
            consumed.add(("k", b))
            if last:
                if b == 0:
                    wait_all(wm_v.at[:, pl.ds(2 * D, 4 * D)], wsem.at[_S_MOD_B])
                mods += [modulation(i) for i in ((2,), (3,), (4, 5))[b]]
        s = s * (DH ** -0.5)
        e = jnp.exp(s - jnp.max(s, axis=-1, keepdims=True))
        denom = jnp.sum(e, axis=-1, keepdims=True)
        p = e.astype(bf16)
        parts = []
        for b in range(NB):
            rows = pl.ds(b * 128, 128)
            need(("v", b), vbuf.at[rows], vsem.at[b])
            parts.append(jax.lax.dot_general(p, vbuf[rows, :], (((1,), (1,)), ((), ())),
                                             preferred_element_type=f32))
            consumed.add(("v", b))
        o = jnp.concatenate(parts, axis=1) / denom
        o = jnp.where(own_head, o, 0.0).astype(bf16)
        need(("w", 0), wo_v.at[pl.ds(off, PR)], wsem.at[_S_WO])
        acc = acc + jnp.dot(o, wo_v[pl.ds(off, PR), :], preferred_element_type=f32)
        advance(_NG + AHEAD - 1)
        return acc, mods

    acc = jax.lax.fori_loop(0, NP - 1, lambda j, a: head_pair(j, a, False)[0], jnp.zeros((ROWS, D), f32))
    acc, (gate_a, shift_b, scale_b, gate_b) = head_pair(NP - 1, acc, True)

    x1 = x + gate_a * jnp.sum(acc, axis=0, keepdims=True)
    h2 = (_layernorm(x1) * (1.0 + scale_b) + shift_b).astype(bf16)
    wait_tail("wg", wg_v, wsem.at[_S_WG])
    g = jnp.dot(h2, wg_v[...], preferred_element_type=f32)
    wait_tail("wu", wu_v, wsem.at[_S_WU])
    u = jnp.dot(h2, wu_v[...], preferred_element_type=f32)
    gu = (g * u).astype(bf16)
    y = jnp.zeros((ROWS, D), f32)
    for i in range(WD_CHUNKS):
        rows = pl.ds(i * WDC, WDC)
        wait_tail(i, wd_v.at[rows], wdsem.at[i])
        y = y + jnp.dot(gu[:, i * WDC:(i + 1) * WDC], wd_v[rows, :], preferred_element_type=f32)
    out = x1 + gate_b * y
    out_ref[...] = out[0:1].astype(out_ref.dtype).reshape(1, 1, D)


@jax.jit
def pallas_adaLN_cond__sliding_block_cached__glu_gated_bilinear__decode_kernel(
    A_x: jax.Array,
    A_k_cache: jax.Array,
    A_v_cache: jax.Array,
    A_wq: jax.Array,
    A_wo: jax.Array,
    B_x: jax.Array,
    B_w_gate: jax.Array,
    B_w_up: jax.Array,
    B_w_down: jax.Array,
    c: jax.Array,
    w_mod: jax.Array,
):
    del B_x
    bf16 = jnp.bfloat16
    k_t = jnp.transpose(A_k_cache, (0, 1, 3, 2)).reshape(HD, SK)
    v_t = jnp.transpose(A_v_cache, (0, 1, 3, 2)).reshape(HD, SK)
    return pl.pallas_call(
        _kernel,
        in_specs=[pl.BlockSpec(memory_space=pl.ANY)] * 10,
        out_specs=pl.BlockSpec(memory_space=pltpu.VMEM),
        out_shape=jax.ShapeDtypeStruct((1, 1, D), bf16),
        scratch_shapes=[
            pltpu.VMEM((1, 1, D), bf16), pltpu.VMEM((1, D), bf16),
            pltpu.VMEM((PR, WIN), bf16), pltpu.VMEM((PR, WIN), bf16),
            pltpu.VMEM((D, HD), bf16), pltpu.VMEM((HD, D), bf16),
            pltpu.VMEM((D, FF), bf16), pltpu.VMEM((D, FF), bf16), pltpu.VMEM((FF, D), bf16),
            pltpu.VMEM((D, 6 * D), bf16),
            pltpu.SemaphoreType.DMA((NB,)), pltpu.SemaphoreType.DMA((NB,)),
            pltpu.SemaphoreType.DMA((8,)), pltpu.SemaphoreType.DMA((WD_CHUNKS,)),
        ],
        compiler_params=pltpu.CompilerParams(
            vmem_limit_bytes=64 * 2**20,
            disable_bounds_checks=True,
            disable_semaphore_checks=True,
        ),
    )(A_x, c, k_t, v_t, A_wq, A_wo, B_w_gate, B_w_up, B_w_down, w_mod)
```

```python
import jax
import jax.numpy as jnp
import jax.experimental.pallas as pl
import jax.experimental.pallas.tpu as pltpu

D = 640
H = 32
DH = 192
SK = 32768
WIN = min(4096, max(256, SK // 4))
FF = 1536
HD = H * DH
PR = 2 * DH
NP = H // 2
NB = PR // 128
ROWS = 8

KV_COLS = 1024
AHEAD = 3
TAIL_AHEAD = 100
TAIL_STEP = 64
WD_CHUNKS = 6
WDC = FF // WD_CHUNKS


def _streams(nrows, ncols, r, c, k, row0=0, col0=0):
    na, nb = nrows // r, ncols // c
    per = na // k
    runs = [[(row0 + a * r, col0 + b * c) for a in range(s * per, (s + 1) * per) for b in range(nb)]
            for s in range(k)]
    return [runs[s][i] + (r, c, s % 2) for i in range(per * nb) for s in range(k)]


def _pair_groups():
    groups = []
    for s, kind in enumerate("kv"):
        for blk in range(NB):
            groups.append([(kind, blk, blk * 128 + a * 8, b * KV_COLS, 8, KV_COLS, (a + s) % 2)
                           for b in range(WIN // KV_COLS) for a in range(16)])
    wo = [("w", 0) + p for p in _streams(PR, D, 8, D, 2)]
    riders = range(AHEAD - 1, len(groups))
    per = len(wo) // len(riders)
    for n, gi in enumerate(riders):
        extra = wo[n * per:(n + 1) * per]
        step = 2 * (len(groups[gi]) // (2 * (len(extra) + 1)))
        mixed = []
        for m, piece in enumerate(groups[gi]):
            mixed.append(piece)
            if extra and (m + 1) % step == 0:
                mixed.append(extra.pop(0))
        groups[gi] = mixed + extra
    return groups


_GROUPS = _pair_groups()
_NG = len(_GROUPS)
_LAST_GROUP = {(p[0], p[1]): gi for gi, grp in enumerate(_GROUPS) for p in grp}

_S_MOD_A, _S_MOD_B, _S_WQ, _S_WO, _S_WG, _S_WU, _S_X, _S_C = range(8)


def _layernorm(t):
    mean = jnp.mean(t, axis=-1, keepdims=True)
    d = t - mean
    var = jnp.mean(d * d, axis=-1, keepdims=True)
    return d * jax.lax.rsqrt(var + 1e-5)


def _kernel(x_hbm, c_hbm, k_hbm, v_hbm, wq_hbm, wo_hbm, wg_hbm, wu_hbm, wd_hbm, wm_hbm,
            out_ref,
            x_v, c_v, kbuf, vbuf, wq_v, wo_v, wg_v, wu_v, wd_v, wm_v,
            ksem, vsem, wsem, wdsem):
    f32, bf16 = jnp.float32, jnp.bfloat16

    def start(src, dst, sem, sr, sc, dr, dc, r, c, queue):
        pltpu.make_async_copy(src.at[pl.ds(sr, r), pl.ds(sc, c)],
                              dst.at[pl.ds(dr, r), pl.ds(dc, c)], sem).start(priority=queue)

    def wait_all(ref, sem):
        pltpu.make_async_copy(ref, ref, sem).wait()

    def start_weights(pieces):
        for (hbm, vmem, sem, r0, c0, r, c, queue) in pieces:
            start(hbm, vmem, sem, r0, c0, r0, c0, r, c, queue)

    def weight_pieces(hbm, vmem, sem, *geometry, **origin):
        return [(hbm, vmem, sem) + p for p in _streams(*geometry, **origin)]

    def start_pair_group(j, gi):
        row0 = pl.multiple_of(j * PR, 128)
        for (kind, blk, r0, c0, r, c, queue) in _GROUPS[gi]:
            if kind == "k":
                start(k_hbm, kbuf, ksem.at[blk], row0 + r0, SK - WIN + c0, r0, c0, r, c, queue)
            elif kind == "v":
                start(v_hbm, vbuf, vsem.at[blk], row0 + r0, SK - WIN + c0, r0, c0, r, c, queue)
            else:
                start(wo_hbm, wo_v, wsem.at[_S_WO], row0 + r0, c0, row0 + r0, c0, r, c, queue)

    tail = weight_pieces(wg_hbm, wg_v, wsem.at[_S_WG], D, FF, 8, FF, 8)
    tail_end = {"wg": len(tail)}
    tail += weight_pieces(wu_hbm, wu_v, wsem.at[_S_WU], D, FF, 8, FF, 8)
    tail_end["wu"] = len(tail)
    for i in range(WD_CHUNKS):
        tail += weight_pieces(wd_hbm, wd_v, wdsem.at[i], WDC, D, 8, D, 4, row0=i * WDC)
        tail_end[i] = len(tail)
    tail_pos = [0]

    def start_tail_upto(n):
        n = min(n, len(tail))
        if n > tail_pos[0]:
            start_weights(tail[tail_pos[0]:n])
            tail_pos[0] = n

    def wait_tail(key, ref, sem):
        start_tail_upto(tail_end[key] + TAIL_AHEAD)
        wait_all(ref, sem)

    mod_a = weight_pieces(wm_hbm, wm_v, wsem.at[_S_MOD_A], D, 2 * D, 8, 2 * D, 10)
    mod_b = weight_pieces(wm_hbm, wm_v, wsem.at[_S_MOD_B], D, 4 * D, 8, 2 * D, 10, col0=2 * D)
    wq_pieces = weight_pieces(wq_hbm, wq_v, wsem.at[_S_WQ], D, HD, 8, 1024, 10)
    x_copy = pltpu.make_async_copy(x_hbm, x_v, wsem.at[_S_X])
    c_copy = pltpu.make_async_copy(c_hbm, c_v, wsem.at[_S_C])

    start_weights(mod_a[:8])
    x_copy.start()
    c_copy.start()
    start_weights(mod_a[8:])
    start_weights(wq_pieces[:48])
    x_copy.wait()
    c_copy.wait()
    x = jnp.broadcast_to(x_v[0].astype(f32), (ROWS, D))
    cond = jnp.broadcast_to(c_v[...].astype(f32), (ROWS, D))
    silu_c = (cond * jax.nn.sigmoid(cond)).astype(bf16)
    ln_x = _layernorm(x)
    start_weights(wq_pieces[48:144])
    wait_all(wm_v.at[:, pl.ds(0, 2 * D)], wsem.at[_S_MOD_A])
    shift_a = jnp.dot(silu_c, wm_v[:, 0:D], preferred_element_type=f32)
    scale_a = jnp.dot(silu_c, wm_v[:, D:2 * D], preferred_element_type=f32)
    h = (ln_x * (1.0 + scale_a) + shift_a).astype(bf16)
    start_weights(wq_pieces[144:])
    for gi in range(AHEAD - 1):
        start_pair_group(0, gi)
    start_weights(mod_b)
    wait_all(wq_v, wsem.at[_S_WQ])

    prow = jax.lax.broadcasted_iota(jnp.int32, (ROWS, PR), 0)
    pcol = jax.lax.broadcasted_iota(jnp.int32, (ROWS, PR), 1)
    own_head = prow == (pcol >= DH).astype(jnp.int32)

    def head_pair(j, acc, last):
        started = [AHEAD - 1]
        consumed = set()

        def advance(target):
            while started[0] < target:
                n = started[0]
                if n < _NG:
                    start_pair_group(j, n)
                elif last:
                    start_tail_upto(tail_pos[0] + TAIL_STEP)
                else:
                    assert all(p[:2] in consumed for p in _GROUPS[n - _NG])
                    start_pair_group(j + 1, n - _NG)
                started[0] += 1

        def need(key, ref, sem):
            advance(_LAST_GROUP[key] + AHEAD)
            wait_all(ref, sem)

        def modulation(i):
            return jnp.dot(silu_c, wm_v[:, i * D:(i + 1) * D], preferred_element_type=f32)

        off = pl.multiple_of(j * PR, 128)
        q = jnp.dot(h, wq_v[:, pl.ds(off, PR)], preferred_element_type=f32)
        q = jnp.where(own_head, q, 0.0).astype(bf16)
        mods = []
        s = None
        for b in range(NB):
            rows = pl.ds(b * 128, 128)
            need(("k", b), kbuf.at[rows], ksem.at[b])
            part = jnp.dot(q[:, b * 128:(b + 1) * 128], kbuf[rows, :], preferred_element_type=f32)
            s = part if s is None else s + part
            consumed.add(("k", b))
            if last:
                if b == 0:
                    wait_all(wm_v.at[:, pl.ds(2 * D, 4 * D)], wsem.at[_S_MOD_B])
                mods += [modulation(i) for i in ((2,), (3,), (4, 5))[b]]
        s = s * (DH ** -0.5)
        e = jnp.exp(s - jnp.max(s, axis=-1, keepdims=True))
        denom = jnp.sum(e, axis=-1, keepdims=True)
        p = e.astype(bf16)
        parts = []
        for b in range(NB):
            rows = pl.ds(b * 128, 128)
            need(("v", b), vbuf.at[rows], vsem.at[b])
            parts.append(jax.lax.dot_general(p, vbuf[rows, :], (((1,), (1,)), ((), ())),
                                             preferred_element_type=f32))
            consumed.add(("v", b))
        o = jnp.concatenate(parts, axis=1) / denom
        o = jnp.where(own_head, o, 0.0).astype(bf16)
        need(("w", 0), wo_v.at[pl.ds(off, PR)], wsem.at[_S_WO])
        acc = acc + jnp.dot(o, wo_v[pl.ds(off, PR), :], preferred_element_type=f32)
        advance(_NG + AHEAD - 1)
        return acc, mods

    acc = jax.lax.fori_loop(0, NP - 1, lambda j, a: head_pair(j, a, False)[0], jnp.zeros((ROWS, D), f32))
    acc, (gate_a, shift_b, scale_b, gate_b) = head_pair(NP - 1, acc, True)

    x1 = x + gate_a * jnp.sum(acc, axis=0, keepdims=True)
    h2 = (_layernorm(x1) * (1.0 + scale_b) + shift_b).astype(bf16)
    wait_tail("wg", wg_v, wsem.at[_S_WG])
    g = jnp.dot(h2, wg_v[...], preferred_element_type=f32)
    wait_tail("wu", wu_v, wsem.at[_S_WU])
    u = jnp.dot(h2, wu_v[...], preferred_element_type=f32)
    gu = (g * u).astype(bf16)
    y = jnp.zeros((ROWS, D), f32)
    for i in range(WD_CHUNKS):
        rows = pl.ds(i * WDC, WDC)
        wait_tail(i, wd_v.at[rows], wdsem.at[i])
        y = y + jnp.dot(gu[:, i * WDC:(i + 1) * WDC], wd_v[rows, :], preferred_element_type=f32)
    out = x1 + gate_b * y
    out_ref[...] = out[0:1].astype(out_ref.dtype).reshape(1, 1, D)


def _compiler_params():
    common = dict(vmem_limit_bytes=64 * 2**20, disable_bounds_checks=True)
    try:
        return pltpu.CompilerParams(disable_semaphore_checks=True, **common)
    except TypeError:
        return pltpu.CompilerParams(**common)


@jax.jit
def pallas_adaLN_cond__sliding_block_cached__glu_gated_bilinear__decode_kernel(
    A_x: jax.Array,
    A_k_cache: jax.Array,
    A_v_cache: jax.Array,
    A_wq: jax.Array,
    A_wo: jax.Array,
    B_x: jax.Array,
    B_w_gate: jax.Array,
    B_w_up: jax.Array,
    B_w_down: jax.Array,
    c: jax.Array,
    w_mod: jax.Array,
):
    del B_x
    bf16 = jnp.bfloat16
    k_t = jnp.transpose(A_k_cache, (0, 1, 3, 2)).reshape(HD, SK)
    v_t = jnp.transpose(A_v_cache, (0, 1, 3, 2)).reshape(HD, SK)
    return pl.pallas_call(
        _kernel,
        in_specs=[pl.BlockSpec(memory_space=pl.ANY)] * 10,
        out_specs=pl.BlockSpec(memory_space=pltpu.VMEM),
        out_shape=jax.ShapeDtypeStruct((1, 1, D), bf16),
        scratch_shapes=[
            pltpu.VMEM((1, 1, D), bf16), pltpu.VMEM((1, D), bf16),
            pltpu.VMEM((PR, WIN), bf16), pltpu.VMEM((PR, WIN), bf16),
            pltpu.VMEM((D, HD), bf16), pltpu.VMEM((HD, D), bf16),
            pltpu.VMEM((D, FF), bf16), pltpu.VMEM((D, FF), bf16), pltpu.VMEM((FF, D), bf16),
            pltpu.VMEM((D, 6 * D), bf16),
            pltpu.SemaphoreType.DMA((NB,)), pltpu.SemaphoreType.DMA((NB,)),
            pltpu.SemaphoreType.DMA((8,)), pltpu.SemaphoreType.DMA((WD_CHUNKS,)),
        ],
        compiler_params=_compiler_params(),
    )(A_x, c, k_t, v_t, A_wq, A_wo, B_w_gate, B_w_up, B_w_down, w_mod)
```
